```python
import jax
import jax.numpy as jnp

def _softmax(x, axis=-1):
    return jax.nn.softmax(x, axis=axis)
def _gelu(x):
    return jax.nn.gelu(x, approximate=True)
def _silu(x):
    return jax.nn.silu(x)
def _sigmoid(x):
    return jax.nn.sigmoid(x)
def _layernorm(x, axis=-1, eps=1e-5):
    m = jnp.mean(x, axis=axis, keepdims=True)
    v = jnp.var(x, axis=axis, keepdims=True)
    return (x - m) / jnp.sqrt(v + eps)
def _scatter_add(tgt, idx, src, axis=0):
    return tgt.at[idx].add(src)
def _segment_sum(src, seg, n):
    return jax.ops.segment_sum(src, seg, n)
class _Rng:
    def __init__(self, key):
        self._k = key
    def _next(self):
        self._k, sub = jax.random.split(self._k)
        return sub
    def normal(self, shape):
        return jax.random.normal(self._next(), shape, dtype=jnp.bfloat16)
    def randint(self, lo, hi, shape):
        return jax.random.randint(self._next(), shape, lo, hi, dtype=jnp.int32)
    def uniform(self, shape, lo=0.0, hi=1.0):
        return jax.random.uniform(self._next(), shape, jnp.bfloat16, lo, hi)
    def permutation(self, n):
        return jax.random.permutation(self._next(), n)


kernel_name = 'parallel_sum__sliding_block_cached__moe_arch_mod__decode'

def setup_inputs():
    _rng = _Rng(jax.random.key(int.from_bytes(__import__("os").urandom(4), "little")))
    _w = (lambda a: (lambda t: t.astype(jnp.bfloat16) if jnp.issubdtype(t.dtype, jnp.floating) else t)(jnp.asarray(a)))
    def _A_setup():
        B, Sq, D = 1, 1, 512
        Hq, Hkv, Sk, Dh = 32, 8, 65536, 128
        assert Hq % Hkv == 0, (Hq, Hkv)
        return {
            "x": _w((lambda *s: _rng.normal(s) * 0.05)(B, Sq, D)),
            "k_cache": _w((lambda *s: _rng.normal(s) * 0.05)(B, Hkv, Sk, Dh)),
            "v_cache": _w((lambda *s: _rng.normal(s) * 0.05)(B, Hkv, Sk, Dh)),
            "wq": _w((lambda *s: _rng.normal(s) * 0.05)(D, Hq * Dh) * (D ** -0.5)),
            "wo": _w((lambda *s: _rng.normal(s) * 0.05)(Hq * Dh, D) * ((Hq * Dh) ** -0.5)),
        }
    _A_in = _A_setup()

    def _B_setup():
        B, S, D, F, C = 1, 1, 512, 1792, 1
        return {
            "x": _w((lambda *s: _rng.normal(s) * 0.05)(B, S, D)),
            "w_r": _w((lambda *s: _rng.normal(s) * 0.05)(D)),
            "w_gate": _w((lambda *s: _rng.normal(s) * 0.05)(D, F)),
            "w_up": _w((lambda *s: _rng.normal(s) * 0.05)(D, F)),
            "w_down": _w((lambda *s: _rng.normal(s) * 0.05)(F, D)),
        }
    _B_in = _B_setup()

    return {
        "A_x": _A_in["x"],
        "A_k_cache": _A_in["k_cache"],
        "A_v_cache": _A_in["v_cache"],
        "A_wq": _A_in["wq"],
        "A_wo": _A_in["wo"],
        "B_x": _B_in["x"],
        "B_w_r": _B_in["w_r"],
        "B_w_gate": _B_in["w_gate"],
        "B_w_up": _B_in["w_up"],
        "B_w_down": _B_in["w_down"],
    }

def reference(A_x, A_k_cache, A_v_cache, A_wq, A_wo, B_x, B_w_r, B_w_gate, B_w_up, B_w_down):
    def _A_ref(x, k_cache, v_cache, wq, wo):
        B, Sq, D = x.shape
        Hq, Dh = 32, 128
        Hkv, Sk = k_cache.shape[1], k_cache.shape[2]
        W = min(4096, max(256, Sk // 4))
        rep = Hq // Hkv
        q = (lambda x, *d: x.transpose(*d))((x @ wq).reshape(B, Sq, Hq, Dh), 0, 2, 1, 3)
        k = jnp.repeat(k_cache[:, :, Sk - W:, :], rep, axis=1)
        v = jnp.repeat(v_cache[:, :, Sk - W:, :], rep, axis=1)
        scores = jnp.einsum("bhqd,bhkd->bhqk", q, k) * (Dh ** -0.5)
        p = _softmax(scores, axis=-1)
        o = jnp.einsum("bhqk,bhkd->bhqd", p, v)
        return (lambda x, *d: x.transpose(*d))(o, 0, 2, 1, 3).reshape(B, Sq, Hq * Dh) @ wo

    def _B_ref(x, w_r, w_gate, w_up, w_down):
        B, S, D = x.shape
        C = 1
        r = x @ w_r
        idx = jnp.argsort(-r, axis=-1)[:, :C]
        idx_e = jnp.repeat(idx.reshape(B, C, 1), D, axis=2)
        x_sel = jnp.take_along_axis(x, idx_e, axis=1)
        g = _silu(x_sel @ w_gate)
        u = x_sel @ w_up
        y = (g * u) @ w_down
        r_sel = _sigmoid(jnp.take_along_axis(r, idx, axis=1))
        y = y * r_sel.reshape(B, C, 1)
        b_off = (jnp.arange(B) * S).reshape(B, 1)
        flat_idx = (idx + b_off).reshape(B * C)
        zero = (x * 0.0).reshape(B * S, D)
        upd = _scatter_add(zero, flat_idx, y.reshape(B * C, D), axis=0)
        return x + upd.reshape(B, S, D)

    x = A_x
    xn = _layernorm(x, axis=-1)
    return x + _A_ref(xn, A_k_cache, A_v_cache, A_wq, A_wo) + _B_ref(xn, B_w_r, B_w_gate, B_w_up, B_w_down)
```

```python
import jax
import jax.numpy as jnp
from jax import lax
import jax.experimental.pallas as pl
import jax.experimental.pallas.tpu as pltpu

_HQ, _DH = 32, 128
_NT = (((1,), (1,)), ((), ()))
_bf16, _f32 = jnp.bfloat16, jnp.float32


@jax.jit
def pallas_parallel_sum__sliding_block_cached__moe_arch_mod__decode_kernel(
    A_x: jax.Array,
    A_k_cache: jax.Array,
    A_v_cache: jax.Array,
    A_wq: jax.Array,
    A_wo: jax.Array,
    B_x: jax.Array,
    B_w_r: jax.Array,
    B_w_gate: jax.Array,
    B_w_up: jax.Array,
    B_w_down: jax.Array,
):
    B, Sq, D = A_x.shape
    assert B == 1 and Sq == 1
    HKV, Sk = A_k_cache.shape[1], A_k_cache.shape[2]
    W = min(4096, max(256, Sk // 4))
    REP = _HQ // HKV
    F = B_w_gate.shape[1]
    DH = _DH
    assert REP == 4 and HKV == 8

    def kernel(x_hbm, k_hbm, v_hbm, wq_hbm, wo_hbm, wr_hbm, wg_hbm, wu_hbm, wd_hbm, o_ref,
               xb, wrb, kb, vb, wqb, wob, wgb, wub, wdb, qs, ps, ls, lhs, sems):
        cnt = [0]

        def cp(src, dst):
            c = pltpu.make_async_copy(src, dst, sems.at[cnt[0]])
            cnt[0] += 1
            c.start()
            return c

        c_x = cp(x_hbm, xb)
        c_wr = cp(wr_hbm, wrb)
        c_wq = cp(wq_hbm, wqb)
        c_k = [cp(k_hbm.at[0, pl.ds(4 * i, 4), pl.ds(Sk - W, W)], kb.at[pl.ds(4 * i, 4)]) for i in range(2)]
        c_v = [cp(v_hbm.at[0, pl.ds(4 * i, 4), pl.ds(Sk - W, W)], vb.at[pl.ds(4 * i, 4)]) for i in range(2)]
        c_wo = cp(wo_hbm, wob)
        c_wg = cp(wg_hbm, wgb)
        c_wu = cp(wu_hbm, wub)
        dsp = [(0, 1024), (1024, 512), (1536, 256)]
        c_wd = [cp(wd_hbm.at[pl.ds(s, n)], wdb.at[pl.ds(s, n)]) for s, n in dsp]

        c_x.wait()
        x = xb[0].astype(_f32)
        m = jnp.mean(x, axis=-1, keepdims=True)
        xc = x - m
        var = jnp.mean(xc * xc, axis=-1, keepdims=True)
        xn = xc / jnp.sqrt(var + 1e-5)
        xn_b = xn.astype(_bf16)
        xn8 = jnp.broadcast_to(xn_b, (8, D))
        c_wr.wait()
        wr = wrb[...].reshape(1, D).astype(_f32)
        r = jnp.sum(xn_b.astype(_f32) * wr, axis=-1, keepdims=True)
        rsel = jax.nn.sigmoid(r)

        row = lax.broadcasted_iota(jnp.int32, (8, DH), 0)
        c_wq.wait()
        q_all = jnp.dot(xn8, wqb[...], preferred_element_type=_f32)
        for h in range(HKV):
            b = [q_all[:, (REP * h + g) * DH:(REP * h + g + 1) * DH] for g in range(REP)]
            qh = jnp.where(row == 0, b[0], jnp.where(row == 1, b[1], jnp.where(row == 2, b[2], b[3])))
            qs[h] = qh.astype(_bf16)

        def kbody(h, c):
            s = lax.dot_general(qs[h], kb[h], _NT, preferred_element_type=_f32) * (DH ** -0.5)
            mx = jnp.max(s, axis=-1, keepdims=True)
            p = jnp.exp(s - mx)
            l = jnp.sum(p, axis=-1, keepdims=True)
            ps[h] = p.astype(_bf16)
            ls[h] = jnp.broadcast_to(1.0 / l, (8, DH))
            return c

        for i in range(2):
            c_k[i].wait()
            lax.fori_loop(4 * i, 4 * i + 4, kbody, 0)

        def vbody(h, c):
            o = jnp.dot(ps[h], vb[h], preferred_element_type=_f32) * ls[h]
            parts = [jnp.where(row == g, o, 0.0).astype(_bf16) for g in range(REP)]
            lhs[h] = jnp.concatenate(parts, axis=1)
            return c

        for i in range(2):
            c_v[i].wait()
            lax.fori_loop(4 * i, 4 * i + 4, vbody, 0)

        c_wo.wait()

        def obody(h, acc):
            rows = pl.ds(pl.multiple_of(h * (REP * DH), REP * DH), REP * DH)
            return acc + jnp.dot(lhs[h], wob[rows, :], preferred_element_type=_f32)

        acc = lax.fori_loop(0, HKV, obody, jnp.zeros((8, D), _f32))
        a = jnp.sum(acc, axis=0, keepdims=True)

        c_wg.wait()
        g = jnp.dot(xn8, wgb[...], preferred_element_type=_f32)
        c_wu.wait()
        u = jnp.dot(xn8, wub[...], preferred_element_type=_f32)
        hh = (g * jax.nn.sigmoid(g) * u).astype(_bf16)
        y = jnp.zeros((8, D), _f32)
        for (s, n), c in zip(dsp, c_wd):
            c.wait()
            y = y + jnp.dot(hh[:, s:s + n], wdb[pl.ds(s, n), :], preferred_element_type=_f32)
        out = x + a + xn + y[0:1] * rsel
        o_ref[0] = out.astype(o_ref.dtype)

    any_ = pl.BlockSpec(memory_space=pl.ANY)
    return pl.pallas_call(
        kernel,
        in_specs=[any_] * 9,
        out_specs=pl.BlockSpec(memory_space=pltpu.VMEM),
        out_shape=jax.ShapeDtypeStruct((1, 1, D), A_x.dtype),
        scratch_shapes=[
            pltpu.VMEM((1, 1, D), _bf16), pltpu.VMEM((D,), _bf16),
            pltpu.VMEM((HKV, W, DH), _bf16), pltpu.VMEM((HKV, W, DH), _bf16),
            pltpu.VMEM((D, _HQ * DH), _bf16), pltpu.VMEM((_HQ * DH, D), _bf16),
            pltpu.VMEM((D, F), _bf16), pltpu.VMEM((D, F), _bf16), pltpu.VMEM((F, D), _bf16),
            pltpu.VMEM((HKV, 8, DH), _bf16), pltpu.VMEM((HKV, 8, W), _bf16),
            pltpu.VMEM((HKV, 8, DH), _f32), pltpu.VMEM((HKV, 8, REP * DH), _bf16),
            pltpu.SemaphoreType.DMA((13,)),
        ],
        compiler_params=pltpu.CompilerParams(vmem_limit_bytes=64 * 1024 * 1024),
    )(A_x, A_k_cache, A_v_cache, A_wq, A_wo, B_w_r, B_w_gate, B_w_up, B_w_down)
```

```python
import jax
import jax.numpy as jnp
from jax import lax
import jax.experimental.pallas as pl
import jax.experimental.pallas.tpu as pltpu

_HQ, _DH = 32, 128
_NT = (((1,), (1,)), ((), ()))
_F32 = jnp.float32
_KV_SPLIT = 2
_VPU_TAIL = (128, 64, 32, 16, 16)
_MXU_TAIL = (512, 256)


@jax.jit
def pallas_parallel_sum__sliding_block_cached__moe_arch_mod__decode_kernel(
    A_x: jax.Array,
    A_k_cache: jax.Array,
    A_v_cache: jax.Array,
    A_wq: jax.Array,
    A_wo: jax.Array,
    B_x: jax.Array,
    B_w_r: jax.Array,
    B_w_gate: jax.Array,
    B_w_up: jax.Array,
    B_w_down: jax.Array,
):
    del B_x
    B, Sq, D = A_x.shape
    HKV, Sk = A_k_cache.shape[1], A_k_cache.shape[2]
    F = B_w_gate.shape[1]
    DH = _DH
    W = min(4096, max(256, Sk // 4))
    REP = _HQ // HKV
    HS = HKV // _KV_SPLIT
    wdt = A_x.dtype
    assert B == 1 and Sq == 1 and REP <= 8 and HKV % _KV_SPLIT == 0

    mxu_sz = (F - sum(_MXU_TAIL) - sum(_VPU_TAIL),) + _MXU_TAIL
    sizes = mxu_sz + _VPU_TAIL
    starts = [sum(sizes[:i]) for i in range(len(sizes))]
    n_mxu = len(mxu_sz)
    vpu0 = sum(mxu_sz)
    n_vpu_rows = F - vpu0
    n_sems = 7 + 2 * _KV_SPLIT + len(sizes)

    def kernel(x_hbm, k_hbm, v_hbm, wq_hbm, wo_hbm, wr_hbm, wg_hbm, wu_hbm, wd_hbm, o_hbm,
               xb, wrb, wqb, wob, wgb, wub, qs, ps, ls, lhs, ob, *bufs):
        kb = bufs[:_KV_SPLIT]
        vb = bufs[_KV_SPLIT:2 * _KV_SPLIT]
        wdb = bufs[2 * _KV_SPLIT:]

        def body(sems):
            n_used = [0]

            def start_copy(src, dst):
                c = pltpu.make_async_copy(src, dst, sems.at[n_used[0]])
                n_used[0] += 1
                c.start()
                return c

            win = pl.ds(Sk - W, W)
            c_x = start_copy(x_hbm, xb)
            c_wq = start_copy(wq_hbm, wqb)
            c_wr = start_copy(wr_hbm, wrb)
            c_k = [start_copy(k_hbm.at[0, pl.ds(HS * i, HS), win], kb[i]) for i in range(_KV_SPLIT)]
            c_v = [start_copy(v_hbm.at[0, pl.ds(HS * i, HS), win], vb[i]) for i in range(_KV_SPLIT)]
            c_wo = start_copy(wo_hbm, wob)
            c_wg = start_copy(wg_hbm, wgb)
            c_wu = start_copy(wu_hbm, wub)
            c_wd = [start_copy(wd_hbm.at[pl.ds(s, n)], wdb[i])
                    for i, (s, n) in enumerate(zip(starts, sizes))]

            c_x.wait()
            x = xb[0].astype(_F32)
            xc = x - jnp.mean(x, axis=-1, keepdims=True)
            var = jnp.mean(xc * xc, axis=-1, keepdims=True)
            xn = xc / jnp.sqrt(var + 1e-5)
            xn_b = xn.astype(wdt)
            xn8 = jnp.broadcast_to(xn_b, (8, D))

            row = lax.broadcasted_iota(jnp.int32, (8, DH), 0)
            c_wq.wait()
            q_all = jnp.dot(xn8, wqb[...], preferred_element_type=_F32)
            for h in range(HKV):
                blk = [q_all[:, (REP * h + g) * DH:(REP * h + g + 1) * DH] for g in range(REP)]
                qh = blk[REP - 1]
                for g in range(REP - 2, -1, -1):
                    qh = jnp.where(row == g, blk[g], qh)
                qs[h] = qh.astype(wdt)

            c_wr.wait()
            wr = wrb[...].reshape(1, D).astype(_F32)
            rsel = jax.nn.sigmoid(jnp.sum(xn_b.astype(_F32) * wr, axis=-1, keepdims=True))

            for i in range(_KV_SPLIT):
                def kbody(j, carry, i=i):
                    h = i * HS + j
                    s = lax.dot_general(qs[h], kb[i][j], _NT, preferred_element_type=_F32)
                    s = s * (DH ** -0.5)
                    p = jnp.exp(s - jnp.max(s, axis=-1, keepdims=True))
                    ps[h] = p.astype(wdt)
                    ls[h] = jnp.broadcast_to(1.0 / jnp.sum(p, axis=-1, keepdims=True), (8, DH))
                    return carry

                c_k[i].wait()
                lax.fori_loop(0, HS, kbody, 0)

            for i in range(_KV_SPLIT):
                def vbody(j, carry, i=i):
                    h = i * HS + j
                    o = jnp.dot(ps[h], vb[i][j], preferred_element_type=_F32) * ls[h]
                    lhs[h] = jnp.concatenate(
                        [jnp.where(row == g, o, 0.0).astype(wdt) for g in range(REP)], axis=1)
                    return carry

                c_v[i].wait()
                lax.fori_loop(0, HS, vbody, 0)

            c_wo.wait()

            def obody(h, acc):
                rows = pl.ds(pl.multiple_of(h * (REP * DH), REP * DH), REP * DH)
                return acc + jnp.dot(lhs[h], wob[rows, :], preferred_element_type=_F32)

            acc = lax.fori_loop(0, HKV, obody, jnp.zeros((8, D), _F32))
            row0 = lax.broadcasted_iota(jnp.int32, (8, D), 0) == 0
            acc = acc + jnp.where(row0, jnp.broadcast_to(x + xn, (8, D)), 0.0)

            c_wg.wait()
            g = jnp.dot(xn8, wgb[...], preferred_element_type=_F32)
            c_wu.wait()
            u = jnp.dot(xn8, wub[...], preferred_element_type=_F32)
            hh = (g * jax.nn.sigmoid(g) * u).astype(wdt)
            ht = jnp.broadcast_to(hh[0:1, vpu0:].astype(_F32), (DH, n_vpu_rows)).T * rsel
            y = jnp.zeros((8, D), _F32)
            for i in range(n_mxu):
                c_wd[i].wait()
                y = y + jnp.dot(hh[:, starts[i]:starts[i] + sizes[i]], wdb[i][...],
                                preferred_element_type=_F32)
            acc = acc + jnp.where(row0, y * rsel, 0.0)
            for i in range(n_mxu, len(sizes)):
                s, n = starts[i] - vpu0, sizes[i]
                c_wd[i].wait()
                prod = wdb[i][...].astype(_F32) * jnp.concatenate([ht[s:s + n]] * (D // DH), axis=1)
                acc = acc + jnp.sum(prod.reshape(n // 8, 8, D), axis=0)

            ob[0] = jnp.sum(acc, axis=0, keepdims=True).astype(ob.dtype)
            start_copy(ob, o_hbm).wait()

        pl.run_scoped(body, pltpu.SemaphoreType.DMA((n_sems,)))

    hbm = pl.BlockSpec(memory_space=pl.ANY)
    return pl.pallas_call(
        kernel,
        in_specs=[hbm] * 9,
        out_specs=hbm,
        out_shape=jax.ShapeDtypeStruct((B, Sq, D), wdt),
        scratch_shapes=[
            pltpu.VMEM((B, Sq, D), wdt),
            pltpu.VMEM((D,), wdt),
            pltpu.VMEM((D, _HQ * DH), wdt),
            pltpu.VMEM((_HQ * DH, D), wdt),
            pltpu.VMEM((D, F), wdt),
            pltpu.VMEM((D, F), wdt),
            pltpu.VMEM((HKV, 8, DH), wdt),
            pltpu.VMEM((HKV, 8, W), wdt),
            pltpu.VMEM((HKV, 8, DH), _F32),
            pltpu.VMEM((HKV, 8, REP * DH), wdt),
            pltpu.VMEM((B, Sq, D), wdt),
        ] + [pltpu.VMEM((HS, W, DH), wdt)] * (2 * _KV_SPLIT)
          + [pltpu.VMEM((n, D), wdt) for n in sizes],
        compiler_params=pltpu.CompilerParams(vmem_limit_bytes=64 * 1024 * 1024),
    )(A_x, A_k_cache, A_v_cache, A_wq, A_wo, B_w_r, B_w_gate, B_w_up, B_w_down)
```

```python
import jax
import jax.numpy as jnp
from jax import lax
import jax.experimental.pallas as pl
import jax.experimental.pallas.tpu as pltpu

_HQ, _DH = 32, 128
_NT = (((1,), (1,)), ((), ()))
_F32 = jnp.float32
_KV_SPLIT = 2
_WO_SPLIT = 4
_HOP = ((128, None, "wq"), (128, "wq", "k0"), (128, "k0", "k1"),
        (128, "k1", "wg"), (128, "wu", "v0"), (128, "v0", "v1"))
_HOP_USE = "wo2"
_MXU_TAIL = 256
_VPU_TAIL = (128, 64, 32, 16, 16)


def _offsets(sizes, base=0):
    return [base + sum(sizes[:i]) for i in range(len(sizes))]


@jax.jit
def pallas_parallel_sum__sliding_block_cached__moe_arch_mod__decode_kernel(
    A_x: jax.Array,
    A_k_cache: jax.Array,
    A_v_cache: jax.Array,
    A_wq: jax.Array,
    A_wo: jax.Array,
    B_x: jax.Array,
    B_w_r: jax.Array,
    B_w_gate: jax.Array,
    B_w_up: jax.Array,
    B_w_down: jax.Array,
):
    del B_x
    B, Sq, D = A_x.shape
    HKV, Sk = A_k_cache.shape[1], A_k_cache.shape[2]
    F = B_w_gate.shape[1]
    DH = _DH
    W = min(4096, max(256, Sk // 4))
    REP = _HQ // HKV
    HS = HKV // _KV_SPLIT
    HO = HKV // _WO_SPLIT
    wdt = A_x.dtype
    assert B == 1 and Sq == 1 and REP <= 8
    assert HKV % _KV_SPLIT == 0 and HKV % _WO_SPLIT == 0

    hop_sz = tuple(h[0] for h in _HOP)
    hop_st = _offsets(hop_sz)
    n_hop_rows = sum(hop_sz)
    mxu_sz = (F - n_hop_rows - _MXU_TAIL - sum(_VPU_TAIL), _MXU_TAIL)
    sizes = mxu_sz + _VPU_TAIL
    starts = _offsets(sizes, n_hop_rows)
    n_mxu = len(mxu_sz)
    vpu0 = starts[n_mxu]
    n_vpu_rows = F - vpu0
    n_sems = 6 + 2 * _KV_SPLIT + _WO_SPLIT + len(sizes) + 2 * len(_HOP)

    def kernel(x_hbm, k_hbm, v_hbm, wq_hbm, wo_hbm, wr_hbm, wg_hbm, wu_hbm, wd_hbm, o_hbm,
               xb, wrb, wqb, wgb, wub, qs, ps, ls, lhs, hs, hts, wdh, ob, *bufs):
        bufs = list(bufs)

        def take(n):
            return [bufs.pop(0) for _ in range(n)]

        kb, vb, wob = take(_KV_SPLIT), take(_KV_SPLIT), take(_WO_SPLIT)
        wdb, smb = take(len(sizes)), take(len(_HOP))

        def body(sems):
            n_used = [0]

            def make_copy(src, dst):
                c = pltpu.make_async_copy(src, dst, sems.at[n_used[0]])
                n_used[0] += 1
                return c

            def start_copy(src, dst):
                c = make_copy(src, dst)
                c.start()
                return c

            h2s = [make_copy(wd_hbm.at[pl.ds(s, n)], smb[i])
                   for i, (s, n) in enumerate(zip(hop_st, hop_sz))]
            s2v = [make_copy(smb[i], wdh.at[pl.ds(s, n)])
                   for i, (s, n) in enumerate(zip(hop_st, hop_sz))]

            def hop_start(name):
                for i, h in enumerate(_HOP):
                    if h[1] == name:
                        h2s[i].start()

            win = pl.ds(Sk - W, W)
            main = {}
            c_x = start_copy(x_hbm, xb)
            main["wq"] = start_copy(wq_hbm, wqb)
            hop_start(None)
            c_wr = start_copy(wr_hbm, wrb)
            for i in range(_KV_SPLIT):
                main["k%d" % i] = start_copy(k_hbm.at[0, pl.ds(HS * i, HS), win], kb[i])
            main["wg"] = start_copy(wg_hbm, wgb)
            main["wu"] = start_copy(wu_hbm, wub)
            for i in range(_KV_SPLIT):
                main["v%d" % i] = start_copy(v_hbm.at[0, pl.ds(HS * i, HS), win], vb[i])
            for i in range(_WO_SPLIT):
                n = HO * REP * DH
                main["wo%d" % i] = start_copy(wo_hbm.at[pl.ds(i * n, n)], wob[i])
            for i, (s, n) in enumerate(zip(starts, sizes)):
                main["wd%d" % i] = start_copy(wd_hbm.at[pl.ds(s, n)], wdb[i])

            def wait_main(name):
                for i, h in enumerate(_HOP):
                    if h[2] == name:
                        h2s[i].wait()
                        s2v[i].start()
                main[name].wait()
                hop_start(name)

            c_x.wait()
            x = xb[0].astype(_F32)
            xc = x - jnp.mean(x, axis=-1, keepdims=True)
            var = jnp.mean(xc * xc, axis=-1, keepdims=True)
            xn = xc / jnp.sqrt(var + 1e-5)
            xn_b = xn.astype(wdt)
            xn8 = jnp.broadcast_to(xn_b, (8, D))

            row = lax.broadcasted_iota(jnp.int32, (8, DH), 0)
            wait_main("wq")
            q_all = jnp.dot(xn8, wqb[...], preferred_element_type=_F32)
            for h in range(HKV):
                blk = [q_all[:, (REP * h + g) * DH:(REP * h + g + 1) * DH] for g in range(REP)]
                qh = blk[REP - 1]
                for g in range(REP - 2, -1, -1):
                    qh = jnp.where(row == g, blk[g], qh)
                qs[h] = qh.astype(wdt)

            c_wr.wait()
            wr = wrb[...].reshape(1, D).astype(_F32)
            rsel = jax.nn.sigmoid(jnp.sum(xn_b.astype(_F32) * wr, axis=-1, keepdims=True))

            for i in range(_KV_SPLIT):
                def kbody(j, carry, i=i):
                    h = i * HS + j
                    s = lax.dot_general(qs[h], kb[i][j], _NT, preferred_element_type=_F32)
                    s = s * (DH ** -0.5)
                    p = jnp.exp(s - jnp.max(s, axis=-1, keepdims=True))
                    ps[h] = p.astype(wdt)
                    ls[h] = jnp.broadcast_to(1.0 / jnp.sum(p, axis=-1, keepdims=True), (8, DH))
                    return carry

                wait_main("k%d" % i)
                lax.fori_loop(0, HS, kbody, 0)

            wait_main("wg")
            g = jnp.dot(xn8, wgb[...], preferred_element_type=_F32)
            wait_main("wu")
            u = jnp.dot(xn8, wub[...], preferred_element_type=_F32)
            hh = (g * jax.nn.sigmoid(g) * u).astype(wdt)
            hs[...] = hh
            hts[...] = jnp.broadcast_to(hh[0:1, vpu0:].astype(_F32), (DH, n_vpu_rows)).T * rsel

            for i in range(_KV_SPLIT):
                def vbody(j, carry, i=i):
                    h = i * HS + j
                    o = jnp.dot(ps[h], vb[i][j], preferred_element_type=_F32) * ls[h]
                    lhs[h] = jnp.concatenate(
                        [jnp.where(row == g, o, 0.0).astype(wdt) for g in range(REP)], axis=1)
                    return carry

                wait_main("v%d" % i)
                lax.fori_loop(0, HS, vbody, 0)

            row0 = lax.broadcasted_iota(jnp.int32, (8, D), 0) == 0
            acc = jnp.where(row0, jnp.broadcast_to(x + xn, (8, D)), 0.0)
            y = None
            for i in range(_WO_SPLIT):
                wait_main("wo%d" % i)
                o_rows = jnp.concatenate([lhs[i * HO + j] for j in range(HO)], axis=1)
                acc = acc + jnp.dot(o_rows, wob[i][...], preferred_element_type=_F32)
                if _HOP_USE == "wo%d" % i:
                    for c in s2v:
                        c.wait()
                    y = jnp.dot(hs[:, :n_hop_rows], wdh[...], preferred_element_type=_F32)
            for i in range(n_mxu):
                wait_main("wd%d" % i)
                y = y + jnp.dot(hs[:, starts[i]:starts[i] + sizes[i]], wdb[i][...],
                                preferred_element_type=_F32)
            acc = acc + jnp.where(row0, y * rsel, 0.0)
            for i in range(n_mxu, len(sizes)):
                s, n = starts[i] - vpu0, sizes[i]
                hcol = jnp.concatenate([hts[s:s + n]] * (D // DH), axis=1)
                wait_main("wd%d" % i)
                prod = wdb[i][...].astype(_F32) * hcol
                acc = acc + jnp.sum(prod.reshape(n // 8, 8, D), axis=0)

            ob[0] = jnp.sum(acc, axis=0, keepdims=True).astype(ob.dtype)
            start_copy(ob, o_hbm).wait()

        pl.run_scoped(body, pltpu.SemaphoreType.DMA((n_sems,)))

    hbm = pl.BlockSpec(memory_space=pl.ANY)
    return pl.pallas_call(
        kernel,
        in_specs=[hbm] * 9,
        out_specs=hbm,
        out_shape=jax.ShapeDtypeStruct((B, Sq, D), wdt),
        scratch_shapes=[
            pltpu.VMEM((B, Sq, D), wdt),
            pltpu.VMEM((D,), wdt),
            pltpu.VMEM((D, _HQ * DH), wdt),
            pltpu.VMEM((D, F), wdt),
            pltpu.VMEM((D, F), wdt),
            pltpu.VMEM((HKV, 8, DH), wdt),
            pltpu.VMEM((HKV, 8, W), wdt),
            pltpu.VMEM((HKV, 8, DH), _F32),
            pltpu.VMEM((HKV, 8, REP * DH), wdt),
            pltpu.VMEM((8, F), wdt),
            pltpu.VMEM((n_vpu_rows, DH), _F32),
            pltpu.VMEM((n_hop_rows, D), wdt),
            pltpu.VMEM((B, Sq, D), wdt),
        ] + [pltpu.VMEM((HS, W, DH), wdt)] * (2 * _KV_SPLIT)
          + [pltpu.VMEM((HO * REP * DH, D), wdt)] * _WO_SPLIT
          + [pltpu.VMEM((n, D), wdt) for n in sizes]
          + [pltpu.SMEM((n, D), wdt) for n in hop_sz],
        compiler_params=pltpu.CompilerParams(vmem_limit_bytes=64 * 1024 * 1024),
    )(A_x, A_k_cache, A_v_cache, A_wq, A_wo, B_w_r, B_w_gate, B_w_up, B_w_down)
```

```python
import jax
import jax.numpy as jnp
from jax import lax
import jax.experimental.pallas as pl
import jax.experimental.pallas.tpu as pltpu

_HQ, _DH = 32, 128
_NT = (((1,), (1,)), ((), ()))
_F32 = jnp.float32
_KV_SPLIT = 2
_WO_SPLIT = 4
_HOP = ((256, "wq", "wo0"), (256, "k1", "wo0"), (256, "v0", "wo2"), (128, "v1", "wo3"))
_MXU_TAIL = 256
_VPU_TAIL = (128, 64, 32, 16, 16)


def _offsets(sizes, base=0):
    return [base + sum(sizes[:i]) for i in range(len(sizes))]


@jax.jit
def pallas_parallel_sum__sliding_block_cached__moe_arch_mod__decode_kernel(
    A_x: jax.Array,
    A_k_cache: jax.Array,
    A_v_cache: jax.Array,
    A_wq: jax.Array,
    A_wo: jax.Array,
    B_x: jax.Array,
    B_w_r: jax.Array,
    B_w_gate: jax.Array,
    B_w_up: jax.Array,
    B_w_down: jax.Array,
):
    del B_x
    B, Sq, D = A_x.shape
    HKV, Sk = A_k_cache.shape[1], A_k_cache.shape[2]
    F = B_w_gate.shape[1]
    DH = _DH
    W = min(4096, max(256, Sk // 4))
    REP = _HQ // HKV
    HS = HKV // _KV_SPLIT
    HO = HKV // _WO_SPLIT
    wdt = A_x.dtype
    assert B == 1 and Sq == 1 and REP <= 8
    assert HKV % _KV_SPLIT == 0 and HKV % _WO_SPLIT == 0

    hop_sz = tuple(h[0] for h in _HOP)
    hop_st = _offsets(hop_sz)
    n_hop_rows = sum(hop_sz)
    mxu_sz = (F - n_hop_rows - _MXU_TAIL - sum(_VPU_TAIL), _MXU_TAIL)
    sizes = mxu_sz + _VPU_TAIL
    starts = _offsets(sizes, n_hop_rows)
    n_mxu = len(mxu_sz)
    vpu0 = starts[n_mxu]
    n_vpu_rows = F - vpu0
    n_sems = 6 + 2 * _KV_SPLIT + _WO_SPLIT + len(sizes) + 2 * len(_HOP)

    def kernel(x_hbm, k_hbm, v_hbm, wq_hbm, wo_hbm, wr_hbm, wg_hbm, wu_hbm, wd_hbm, o_hbm,
               xb, wrb, wqb, wgb, wub, qs, ps, ls, lhs, hs, hts, ob, *bufs):
        bufs = list(bufs)

        def take(n):
            return [bufs.pop(0) for _ in range(n)]

        kb, vb, wob = take(_KV_SPLIT), take(_KV_SPLIT), take(_WO_SPLIT)
        wdb, wdh, smb = take(len(sizes)), take(len(_HOP)), take(len(_HOP))

        def body(sems):
            n_used = [0]

            def make_copy(src, dst):
                c = pltpu.make_async_copy(src, dst, sems.at[n_used[0]])
                n_used[0] += 1
                return c

            def start_copy(src, dst):
                c = make_copy(src, dst)
                c.start()
                return c

            win = pl.ds(Sk - W, W)
            main = {}
            c_x = start_copy(x_hbm, xb)
            main["wq"] = start_copy(wq_hbm, wqb)
            h2s = [start_copy(wd_hbm.at[pl.ds(s, n)], smb[i])
                   for i, (s, n) in enumerate(zip(hop_st, hop_sz))]
            s2v = [make_copy(smb[i], wdh[i]) for i in range(len(_HOP))]
            c_wr = start_copy(wr_hbm, wrb)
            for i in range(_KV_SPLIT):
                main["k%d" % i] = start_copy(k_hbm.at[0, pl.ds(HS * i, HS), win], kb[i])
            main["wg"] = start_copy(wg_hbm, wgb)
            main["wu"] = start_copy(wu_hbm, wub)
            for i in range(_KV_SPLIT):
                main["v%d" % i] = start_copy(v_hbm.at[0, pl.ds(HS * i, HS), win], vb[i])
            for i in range(_WO_SPLIT):
                n = HO * REP * DH
                main["wo%d" % i] = start_copy(wo_hbm.at[pl.ds(i * n, n)], wob[i])
            for i, (s, n) in enumerate(zip(starts, sizes)):
                main["wd%d" % i] = start_copy(wd_hbm.at[pl.ds(s, n)], wdb[i])

            def wait_main(name):
                for i, h in enumerate(_HOP):
                    if h[1] == name:
                        h2s[i].wait()
                        s2v[i].start()
                main[name].wait()

            c_x.wait()
            x = xb[0].astype(_F32)
            xc = x - jnp.mean(x, axis=-1, keepdims=True)
            var = jnp.mean(xc * xc, axis=-1, keepdims=True)
            xn = xc / jnp.sqrt(var + 1e-5)
            xn_b = xn.astype(wdt)
            xn8 = jnp.broadcast_to(xn_b, (8, D))

            row = lax.broadcasted_iota(jnp.int32, (8, DH), 0)
            wait_main("wq")
            q_all = jnp.dot(xn8, wqb[...], preferred_element_type=_F32)
            for h in range(HKV):
                blk = [q_all[:, (REP * h + g) * DH:(REP * h + g + 1) * DH] for g in range(REP)]
                qh = blk[REP - 1]
                for g in range(REP - 2, -1, -1):
                    qh = jnp.where(row == g, blk[g], qh)
                qs[h] = qh.astype(wdt)

            c_wr.wait()
            wr = wrb[...].reshape(1, D).astype(_F32)
            rsel = jax.nn.sigmoid(jnp.sum(xn_b.astype(_F32) * wr, axis=-1, keepdims=True))

            for i in range(_KV_SPLIT):
                def kbody(j, carry, i=i):
                    h = i * HS + j
                    s = lax.dot_general(qs[h], kb[i][j], _NT, preferred_element_type=_F32)
                    s = s * (DH ** -0.5)
                    p = jnp.exp(s - jnp.max(s, axis=-1, keepdims=True))
                    ps[h] = p.astype(wdt)
                    ls[h] = jnp.broadcast_to(1.0 / jnp.sum(p, axis=-1, keepdims=True), (8, DH))
                    return carry

                wait_main("k%d" % i)
                lax.fori_loop(0, HS, kbody, 0)

            wait_main("wg")
            gate = jnp.dot(xn8, wgb[...], preferred_element_type=_F32)
            wait_main("wu")
            up = jnp.dot(xn8, wub[...], preferred_element_type=_F32)
            hh = (gate * jax.nn.sigmoid(gate) * up).astype(wdt)
            hs[...] = hh
            hts[...] = jnp.broadcast_to(hh[0:1, vpu0:].astype(_F32), (DH, n_vpu_rows)).T * rsel

            for i in range(_KV_SPLIT):
                def vbody(j, carry, i=i):
                    h = i * HS + j
                    o = jnp.dot(ps[h], vb[i][j], preferred_element_type=_F32) * ls[h]
                    lhs[h] = jnp.concatenate(
                        [jnp.where(row == g, o, 0.0).astype(wdt) for g in range(REP)], axis=1)
                    return carry

                wait_main("v%d" % i)
                lax.fori_loop(0, HS, vbody, 0)

            row0 = lax.broadcasted_iota(jnp.int32, (8, D), 0) == 0
            acc = jnp.where(row0, jnp.broadcast_to(x + xn, (8, D)), 0.0)
            y = jnp.zeros((8, D), _F32)
            for i in range(_WO_SPLIT):
                wait_main("wo%d" % i)
                o_rows = jnp.concatenate([lhs[i * HO + j] for j in range(HO)], axis=1)
                acc = acc + jnp.dot(o_rows, wob[i][...], preferred_element_type=_F32)
                for j, h in enumerate(_HOP):
                    if h[2] == "wo%d" % i:
                        s2v[j].wait()
                        y = y + jnp.dot(hs[:, hop_st[j]:hop_st[j] + hop_sz[j]], wdh[j][...],
                                        preferred_element_type=_F32)
            for i in range(n_mxu):
                wait_main("wd%d" % i)
                y = y + jnp.dot(hs[:, starts[i]:starts[i] + sizes[i]], wdb[i][...],
                                preferred_element_type=_F32)
            acc = acc + jnp.where(row0, y * rsel, 0.0)
            for i in range(n_mxu, len(sizes)):
                s, n = starts[i] - vpu0, sizes[i]
                hcol = jnp.concatenate([hts[s:s + n]] * (D // DH), axis=1)
                wait_main("wd%d" % i)
                prod = wdb[i][...].astype(_F32) * hcol
                acc = acc + jnp.sum(prod.reshape(n // 8, 8, D), axis=0)

            ob[0] = jnp.sum(acc, axis=0, keepdims=True).astype(ob.dtype)
            start_copy(ob, o_hbm).wait()

        pl.run_scoped(body, pltpu.SemaphoreType.DMA((n_sems,)))

    hbm = pl.BlockSpec(memory_space=pl.ANY)
    return pl.pallas_call(
        kernel,
        in_specs=[hbm] * 9,
        out_specs=hbm,
        out_shape=jax.ShapeDtypeStruct((B, Sq, D), wdt),
        scratch_shapes=[
            pltpu.VMEM((B, Sq, D), wdt),
            pltpu.VMEM((D,), wdt),
            pltpu.VMEM((D, _HQ * DH), wdt),
            pltpu.VMEM((D, F), wdt),
            pltpu.VMEM((D, F), wdt),
            pltpu.VMEM((HKV, 8, DH), wdt),
            pltpu.VMEM((HKV, 8, W), wdt),
            pltpu.VMEM((HKV, 8, DH), _F32),
            pltpu.VMEM((HKV, 8, REP * DH), wdt),
            pltpu.VMEM((8, F), wdt),
            pltpu.VMEM((n_vpu_rows, DH), _F32),
            pltpu.VMEM((B, Sq, D), wdt),
        ] + [pltpu.VMEM((HS, W, DH), wdt)] * (2 * _KV_SPLIT)
          + [pltpu.VMEM((HO * REP * DH, D), wdt)] * _WO_SPLIT
          + [pltpu.VMEM((n, D), wdt) for n in sizes]
          + [pltpu.VMEM((n, D), wdt) for n in hop_sz]
          + [pltpu.SMEM((n, D), wdt) for n in hop_sz],
        compiler_params=pltpu.CompilerParams(vmem_limit_bytes=64 * 1024 * 1024),
    )(A_x, A_k_cache, A_v_cache, A_wq, A_wo, B_w_r, B_w_gate, B_w_up, B_w_down)
```
